```python
import os as _os
_os.environ.setdefault("JAX_PLATFORMS", "cpu")
import jax
import jax.numpy as jnp

def _softmax(x, axis=-1):
    return jax.nn.softmax(x, axis=axis)
def _gelu(x):
    return jax.nn.gelu(x, approximate=True)
def _silu(x):
    return jax.nn.silu(x)
def _sigmoid(x):
    return jax.nn.sigmoid(x)
def _layernorm(x, axis=-1, eps=1e-5):
    m = jnp.mean(x, axis=axis, keepdims=True)
    v = jnp.var(x, axis=axis, keepdims=True)
    return (x - m) / jnp.sqrt(v + eps)
def _scatter_add(tgt, idx, src, axis=0):
    return tgt.at[idx].add(src)
def _segment_sum(src, seg, n):
    return jax.ops.segment_sum(src, seg, n)
class _Rng:
    def __init__(self, key):
        self._k = key
    def _next(self):
        self._k, sub = jax.random.split(self._k)
        return sub
    def normal(self, shape):
        return jax.random.normal(self._next(), shape, dtype=jnp.bfloat16)
    def randint(self, lo, hi, shape):
        return jax.random.randint(self._next(), shape, lo, hi, dtype=jnp.int32)
    def uniform(self, shape, lo=0.0, hi=1.0):
        return jax.random.uniform(self._next(), shape, jnp.bfloat16, lo, hi)
    def permutation(self, n):
        return jax.random.permutation(self._next(), n)


kernel_name = 'standalone__seq2seq_rnn_t_joint__speech'

def setup_inputs():
    _rng = _Rng(jax.random.key(int.from_bytes(__import__("os").urandom(4), "little")))
    _w = (lambda a: (lambda t: t.astype(jnp.bfloat16) if jnp.issubdtype(t.dtype, jnp.floating) else t)(jnp.asarray(a)))
    B, T, D, K = 2, 1000, 512, 31
    U = 8
    sc = (1.0 / (K * D)) ** 0.5
    sd = (1.0 / D) ** 0.5
    return {
        "x": _w((lambda *s: _rng.normal(s) * 0.4)(B, T, D) * 0.5),
        "w1": _w((lambda *s: _rng.normal(s) * 1.6)(K, D, D) * sc),
        "w2": _w((lambda *s: _rng.normal(s) * 1.6)(K, D, D) * sc),
        "g": _w((lambda *s: _rng.normal(s) * 1.6)(B, U, D) * 0.5),
        "w_f": _w((lambda *s: _rng.normal(s) * 1.6)(D, D) * sd),
        "w_g": _w((lambda *s: _rng.normal(s) * 1.6)(D, D) * sd),
        "w_o": _w((lambda *s: _rng.normal(s) * 1.6)(D, D) * sd),
    }

def reference(x, w1, w2, g, w_f, w_g, w_o):
    B, T, D = x.shape
    K = w1.shape[0]
    pad = K // 2
    xp = jnp.pad(x, ((0,0),(pad,pad),(0,0)))
    h = jnp.zeros_like(x)
    for i in range(K):
        h = h + jnp.einsum("btc,cd->btd", xp[:, i:i+T, :], w1[i])
    h = _gelu(h)[:, ::2, :]
    T1 = h.shape[1]
    hp = jnp.pad(h, ((0,0),(pad,pad),(0,0)))
    f = jnp.zeros_like(h)
    for i in range(K):
        f = f + jnp.einsum("btc,cd->btd", hp[:, i:i+T1, :], w2[i])
    f = _gelu(f)[:, ::2, :]
    fe = jnp.einsum("btd,de->bte", f, w_f)
    ge = jnp.einsum("bud,de->bue", g, w_g)
    j = jnp.tanh(fe[:, :, None, :] + ge[:, None, :, :])
    return jnp.einsum("btud,dv->btuv", j, w_o)
```

```python
import math

import jax
import jax.numpy as jnp
import jax.experimental.pallas as pl
import jax.experimental.pallas.tpu as pltpu

F32 = jnp.float32
BF16 = jnp.bfloat16

D = 512
NT = D // 128
L1 = 4
L2 = 3
M1 = 1 << L1
M2 = 1 << L2
R1 = 3 ** L1
R2 = 3 ** L2
G2 = 16 // M2
RH = max(R1, R2 * G2)
WR1, WR2, WH0 = 0, 16 * NT, 32 * NT
NB = 32


def _xhat(d, lvl):
    if lvl == 0:
        return [d[0]]
    s = 1 << (lvl - 1)
    d0, d1, d2 = d[0:2 * s - 1], d[s:3 * s - 1], d[2 * s:4 * s - 1]
    return (_xhat([a - b for a, b in zip(d0, d1)], lvl - 1) + _xhat(d1, lvl - 1)
            + _xhat([a - b for a, b in zip(d2, d1)], lvl - 1))


def _what(g, lvl):
    if lvl == 0:
        return [g[0]]
    s = 1 << (lvl - 1)
    lo, hi = g[:s], g[s:]
    return (_what(lo, lvl - 1) + _what([a + b for a, b in zip(lo, hi)], lvl - 1)
            + _what(hi, lvl - 1))


def _yout(p, lvl):
    if lvl == 0:
        return [p[0]]
    n = len(p) // 3
    a, b, c = _yout(p[:n], lvl - 1), _yout(p[n:2 * n], lvl - 1), _yout(p[2 * n:], lvl - 1)
    return [u + v for u, v in zip(a, b)] + [u + v for u, v in zip(b, c)]


def _raw_tap(j, lvl):
    tap = 0
    for k in range(lvl):
        dgt = (j // 3 ** (lvl - 1 - k)) % 3
        if dgt == 1:
            return None
        if dgt == 2:
            tap += 1 << (lvl - 1 - k)
    return tap


def unpk(v):
    return pltpu.bitcast(v, BF16)


def _gelu(x):
    c = math.sqrt(2.0 / math.pi)
    return 0.5 * x * (1.0 + jnp.tanh(c * (x + 0.044715 * (x * x * x))))


def _kernel(x_hbm, w1_hbm, w2_hbm, g_hbm, wf_hbm, wg_hbm, wo_hbm, o_hbm,
            xp, xh1, xh2, wa, wb, acca, accb, tmp, ys, fs, fe_ref, ge_ref,
            g_v, wf_v, wg_v, wo_v, ob, sem_w, sem_m, sem_x, sem_o):
    B, T, _ = x_hbm.shape
    T1 = T // 2
    T2 = T1 // 2
    U = g_hbm.shape[1]

    K = w1_hbm.shape[0]

    ww = (wa, wb)

    class _Copies:
        def __init__(self, cps):
            self.cps = cps

        def start(self):
            for c in self.cps:
                c.start()

        def wait(self, ph):
            for c in (self.cps[:1] if ph == 0 else self.cps[1:]):
                c.wait()

    def w_copy(w_hbm, wr, dt, si):
        c0 = dt * 128 if isinstance(dt, int) else pl.multiple_of(dt * 128, 128)
        n = K // 2
        w2d = w_hbm.at[pl.ds(0, 2 * n)].reshape(n, 2, D, D)
        return _Copies([
            pltpu.make_async_copy(w2d.at[:, 1, :, pl.ds(c0, 128)],
                                  wa.at[pl.ds(wr + 16 * dt, n)], sem_w.at[3 * si]),
            pltpu.make_async_copy(w2d.at[:, 0, :, pl.ds(c0, 128)],
                                  wb.at[pl.ds(wr + 16 * dt, n)], sem_w.at[3 * si + 1]),
            pltpu.make_async_copy(w_hbm.at[2 * n, :, pl.ds(c0, 128)],
                                  wb.at[wr + 16 * dt + n], sem_w.at[3 * si + 2]),
        ])

    xu = x_hbm.bitcast(jnp.uint32)
    x_cps = [pltpu.make_async_copy(xu.at[b, :, pl.ds(ct * 128, 128)],
                                   xp.at[b * NT + ct, pl.ds(8, T1)], sem_x.at[b * NT + ct])
             for b in range(B) for ct in range(NT)]
    small = [pltpu.make_async_copy(s, d_, sem_m.at[1 + k]) for k, (s, d_) in enumerate(
        ((wf_hbm, wf_v), (g_hbm, g_v), (wg_hbm, wg_v), (wo_hbm, wo_v)))]

    z0 = 8 + (T1 // 8) * 8
    for bc in range(B * NT):
        xp[bc, 0:8] = jnp.zeros((8, 128), jnp.uint32)
        xp[bc, z0:] = jnp.zeros((xp.shape[1] - z0, 128), jnp.uint32)
    for c_ in x_cps:
        c_.start()
    w_copy(w1_hbm, WR1, 0, 0).start()
    w_copy(w1_hbm, WR1, 1, 1).start()

    zb = jnp.zeros((512, 128), BF16)
    for dt in range(NT):
        wa[WR1 + 16 * dt + 15] = zb
        wa[WR2 + 16 * dt + 15] = zb
    zf = jnp.zeros((8, 128), F32)
    for ct in range(NT):
        for j in range(M1):
            for b in range(B):
                ys[ct, j, b, 0:8] = zf
                ys[ct, j, b, 8 + NB:16 + NB] = zf
    accb[...] = jnp.zeros(accb.shape, F32)

    for c_ in x_cps:
        c_.wait()
    hm = M1 // 2
    nw = 2 * hm - 1

    def xd(bc, ph, r, l):
        v = xp[bc, pl.ds(r * M1 + l + 1 - ph, 8, stride=M1), :]
        return pltpu.bitcast(v & jnp.uint32(0xFFFF0000) if ph else v << 16, F32)

    def xh1_top(bc, c):
        for r in range(0, NB, 8):
            for ph in range(2):
                for l in range(nw):
                    mid = xd(bc, ph, r, hm + l)
                    tmp[bc, ph, 0, l, r:r + 8] = xd(bc, ph, r, l) - mid
                    tmp[bc, ph, 1, l, r:r + 8] = xd(bc, ph, r, 2 * hm + l) - mid
        return c

    jax.lax.fori_loop(0, B * NT, xh1_top, 0)

    def xh1_rest(i, c):
        bc, hf = i // 2, i % 2
        b, ct = bc // NT, bc % NT
        r = pl.multiple_of(hf * 16, 16)
        r0 = pl.multiple_of(b * NB + hf * 16, 16)
        for ph in range(2):
            for q in range(3):
                if q == 1:
                    dl = [jnp.concatenate([xd(bc, ph, r, hm + l), xd(bc, ph, r + 8, hm + l)], axis=0)
                          for l in range(nw)]
                else:
                    dl = [tmp[bc, ph, q // 2, l, pl.ds(r, 16)] for l in range(nw)]
                for j, v in enumerate(_xhat(dl, L1 - 1)):
                    xh1[ph, q * (R1 // 3) + j, ct, pl.ds(r0, 16)] = v.astype(BF16)
        return c

    jax.lax.fori_loop(0, B * NT * 2, xh1_rest, 0)

    def wt_piece(wr, lvl, dt, ph, buf, p):
        rs = slice(16 * p, 16 * p + 16)
        m = 1 << lvl
        ng = 16 // m
        nr = 3 ** lvl
        for g in range(ng):
            def ld(a):
                return ww[ph][wr + 16 * dt + g * m + a, rs, :].astype(F32)
            for j, v in enumerate(_what([ld(a) for a in range(m)], lvl)):
                if _raw_tap(j, lvl) is None:
                    ww[ph][WH0 + j * ng + g, rs, :] = v.astype(BF16)

    def mm_product(wr, xh, lvl, dt, ph, buf, ab, j):
        m = 1 << lvl
        ng = 16 // m
        raw = _raw_tap(j, lvl)
        res = None
        for g in range(ng):
            lhs = jnp.concatenate([unpk(xh.bitcast(jnp.uint32)[ph, j * ng + g, ct]) for ct in range(NT)], axis=1)
            if raw is not None:
                rhs = unpk(ww[ph].bitcast(jnp.uint32)[wr + 16 * dt + g * m + raw])
            else:
                rhs = unpk(ww[ph].bitcast(jnp.uint32)[WH0 + j * ng + g])
            t = jnp.dot(lhs, rhs, preferred_element_type=F32)
            res = t if res is None else res + t
        if ph == 0:
            acca[j] = res
        else:
            accb[j] = acca[j] + res

    rowid = jax.lax.broadcasted_iota(jnp.int32, (16, 128), 0)

    def epi1(ct, ab, b, hf):
        r0 = b * NB + hf * 16
        y = _yout([accb[j, r0:r0 + 16] for j in range(R1)], L1)
        nfull1 = T1 // M1
        rem1 = T1 % M1
        for j in range(M1):
            h = _gelu(y[j])
            nvalid = nfull1 + (1 if j < rem1 else 0)
            if nvalid < hf * 16 + 16:
                h = jnp.where(rowid[:16] + hf * 16 < nvalid, h, 0.0)
            ys[ct, j, b, 8 + hf * 16:24 + hf * 16] = h

    def xhat2(ct, ph, g, b, hf):
        dd = []
        for l in range(2 * M2 - 1):
            k = 2 * l + (2 if ph == 0 else 1) + 2 * M2 * (g - 1)
            sh = k // M1
            dd.append(ys[ct, k % M1, b, pl.ds(8 + sh + hf * 16, 16), :])
        r0 = b * NB + hf * 16
        for j, v in enumerate(_xhat(dd, L2)):
            xh2[ph, j * G2 + g, ct, r0:r0 + 16] = v.astype(BF16)

    def epi2(ct, ab):
        y = _yout([accb[j] for j in range(R2)], L2)
        for j in range(M2):
            fs[ct, j] = _gelu(y[j]).astype(BF16)

    def interleave(main, fill, head=0):
        for f in main[:head]:
            f()
        main = main[head:]
        nm, nf = len(main), len(fill)
        k = 0
        for i, f in enumerate(main):
            f()
            while k < nf and k * nm < (i + 1) * nf:
                fill[k]()
                k += 1
        while k < nf:
            fill[k]()
            k += 1

    def mix(a, b):
        out = []
        interleave([P(out.append, f) for f in a], [P(out.append, f) for f in b])
        return out

    nreg = [0]

    def region(i, f):
        nreg[0] += 1
        pl.when(i < 2 * NT + nreg[0])(f)

    P = functools_partial
    ord1 = sorted(range(R1), key=lambda j: _raw_tap(j, L1) is None)
    ord2 = sorted(range(R2), key=lambda j: _raw_tap(j, L2) is None)
    nraw1, nraw2 = 0, 0

    w_copy(w1_hbm, WR1, 0, 0).wait(0)
    for p in range(D // 16):
        wt_piece(WR1, L1, 0, 0, 0, p)

    def conv1_body(dt, c):
        ab = dt % 2
        dn = jnp.minimum(dt + 1, NT - 1)
        dp = jnp.maximum(dt - 1, 0)
        d2 = jnp.minimum(dt + 2, NT - 1)

        @pl.when(dt + 2 < NT)
        def _():
            w_copy(w1_hbm, WR1, d2, d2).start()

        @pl.when(dt + 2 == NT)
        def _():
            for c_ in small:
                c_.start()
            w_copy(w2_hbm, WR2, 0, NT).start()

        @pl.when(dt + 1 == NT)
        def _():
            for q in range(1, NT):
                w_copy(w2_hbm, WR2, q, NT + q).start()

        w_copy(w1_hbm, WR1, dt, dt).wait(1)

        fill = [P(wt_piece, WR1, L1, dt, 1, 1, p) for p in range(D // 16)]
        fill = mix(fill, [P(epi1, dp, 1 - ab, b, hf) for b in range(B) for hf in range(2)])
        region(dt, lambda: interleave([P(mm_product, WR1, xh1, L1, dt, 0, 0, ab, j) for j in ord1], fill, nraw1))
        @pl.when(dt + 1 < NT)
        def _():
            w_copy(w1_hbm, WR1, dn, dn).wait(0)

        fill = [P(wt_piece, WR1, L1, dn, 0, 0, p) for p in range(D // 16)]
        fill = mix(fill, [P(xhat2, dp, ph, g, b, hf) for ph in range(2) for g in range(G2)
                          for b in range(B) for hf in range(2)])
        region(dt, lambda: interleave([P(mm_product, WR1, xh1, L1, dt, 1, 1, ab, j) for j in ord1], fill, nraw1))
        return c

    jax.lax.fori_loop(0, NT, conv1_body, 0)

    for b in range(B):
        for hf in range(2):
            epi1(NT - 1, (NT - 1) % 2, b, hf)
    for ph in range(2):
        for g in range(G2):
            for b in range(B):
                for hf in range(2):
                    xhat2(NT - 1, ph, g, b, hf)

    w_copy(w2_hbm, WR2, 0, NT).wait(0)
    for p in range(D // 16):
        wt_piece(WR2, L2, 0, 0, 0, p)

    def conv2_body(dt, c):
        ab = dt % 2
        dn = jnp.minimum(dt + 1, NT - 1)
        dp = jnp.maximum(dt - 1, 0)
        w_copy(w2_hbm, WR2, dt, NT + dt).wait(1)

        fill = [P(wt_piece, WR2, L2, dt, 1, 1, p) for p in range(D // 16)]
        fill.insert(0, P(epi2, dp, 1 - ab))
        region(dt, lambda: interleave([P(mm_product, WR2, xh2, L2, dt, 0, 0, ab, j) for j in ord2], fill, nraw2))
        @pl.when(dt + 1 < NT)
        def _():
            w_copy(w2_hbm, WR2, dn, NT + dn).wait(0)

        fill = [P(wt_piece, WR2, L2, dn, 0, 0, p) for p in range(D // 16)]
        region(dt, lambda: interleave([P(mm_product, WR2, xh2, L2, dt, 1, 1, ab, j) for j in ord2], fill, nraw2))
        return c

    jax.lax.fori_loop(0, NT, conv2_body, 0)
    epi2(NT - 1, (NT - 1) % 2)

    for c_ in small:
        c_.wait()
    f2 = jnp.concatenate([fs[ct].reshape(M2 * B * NB, 128) for ct in range(NT)], axis=1)
    fe_ref[...] = jnp.dot(f2, wf_v[...], preferred_element_type=F32)
    ge_ref[...] = jnp.dot(g_v[...].reshape(B * U, D), wg_v[...], preferred_element_type=F32)

    TC = 64
    ocp = []
    for b in range(B):
        geb = ge_ref[b * U:(b + 1) * U]
        for t0 in range(0, T2, TC):
            tc = min(TC, T2 - t0)
            rows = []
            for t in range(t0, t0 + tc):
                r = (t % M2) * (B * NB) + b * NB + t // M2
                rows.append(jnp.tanh(fe_ref[r:r + 1, :] + geb).astype(BF16))
            jm = jnp.concatenate(rows, axis=0)
            res = jnp.dot(jm, wo_v[...], preferred_element_type=F32)
            ob[b, t0:t0 + tc] = res.astype(BF16).reshape(tc, U, D)
            cp = pltpu.make_async_copy(ob.at[b, pl.ds(t0, tc)], o_hbm.at[b, pl.ds(t0, tc)],
                                       sem_o.at[len(ocp)])
            cp.start()
            ocp.append(cp)
    for cp in ocp:
        cp.wait()


def functools_partial(f, *a):
    return lambda: f(*a)


@jax.jit
def pallas_standalone__seq2seq_rnn_t_joint__speech_kernel(
    x: jax.Array,
    w1: jax.Array,
    w2: jax.Array,
    g: jax.Array,
    w_f: jax.Array,
    w_g: jax.Array,
    w_o: jax.Array,
):
    B, T, Dm = x.shape
    K = w1.shape[0]
    U = g.shape[1]
    assert Dm == D and K == 31 and B == 2 and T % 4 == 0
    T1 = T // 2
    T2 = T1 // 2
    assert -(-T1 // M1) == NB and -(-T2 // M2) == NB
    any_spec = pl.BlockSpec(memory_space=pl.ANY)
    n_out = B * (-(-T2 // 64))
    scratch = [
        pltpu.VMEM((B * NT, M1 * NB + 32, 128), jnp.uint32),
        pltpu.VMEM((2, R1, NT, B * NB, 128), BF16),
        pltpu.VMEM((2, R2 * G2, NT, B * NB, 128), BF16),
        pltpu.VMEM((WH0 + RH, D, 128), BF16),
        pltpu.VMEM((WH0 + RH, D, 128), BF16),
        pltpu.VMEM((R1, B * NB, 128), F32),
        pltpu.VMEM((R1, B * NB, 128), F32),
        pltpu.VMEM((B * NT, 2, 2, M1 - 1, NB, 128), F32),
        pltpu.VMEM((NT, M1, B, NB + 16, 128), F32),
        pltpu.VMEM((NT, M2, B * NB, 128), BF16),
        pltpu.VMEM((M2 * B * NB, D), F32),
        pltpu.VMEM((B * U, D), F32),
        pltpu.VMEM((B, U, D), BF16),
        pltpu.VMEM((D, D), BF16),
        pltpu.VMEM((D, D), BF16),
        pltpu.VMEM((D, D), BF16),
        pltpu.VMEM((B, T2, U, D), BF16),
        pltpu.SemaphoreType.DMA((24,)),
        pltpu.SemaphoreType.DMA((5,)),
        pltpu.SemaphoreType.DMA((B * NT,)),
        pltpu.SemaphoreType.DMA((n_out,)),
    ]
    return pl.pallas_call(
        _kernel,
        in_specs=[any_spec] * 7,
        out_specs=any_spec,
        out_shape=jax.ShapeDtypeStruct((B, T2, U, D), BF16),
        scratch_shapes=scratch,
        compiler_params=pltpu.CompilerParams(vmem_limit_bytes=116 * 1024 * 1024),
    )(x, w1, w2, g, w_f, w_g, w_o)
```

```python
import math

import jax
import jax.numpy as jnp
import jax.experimental.pallas as pl
import jax.experimental.pallas.tpu as pltpu

F32 = jnp.float32
BF16 = jnp.bfloat16

D = 512
NT = D // 128
L1 = 4
L2 = 3
M1 = 1 << L1
M2 = 1 << L2
R1 = 3 ** L1
R2 = 3 ** L2
G2 = 16 // M2
RH = max(R1, R2 * G2)
WR1, WR2, WH0 = 0, 16 * NT, 32 * NT
NB = 32


def _xhat(d, lvl):
    if lvl == 0:
        return [d[0]]
    s = 1 << (lvl - 1)
    d0, d1, d2 = d[0:2 * s - 1], d[s:3 * s - 1], d[2 * s:4 * s - 1]
    return (_xhat([a - b for a, b in zip(d0, d1)], lvl - 1) + _xhat(d1, lvl - 1)
            + _xhat([a - b for a, b in zip(d2, d1)], lvl - 1))


def _what(g, lvl):
    if lvl == 0:
        return [g[0]]
    s = 1 << (lvl - 1)
    lo, hi = g[:s], g[s:]
    return (_what(lo, lvl - 1) + _what([a + b for a, b in zip(lo, hi)], lvl - 1)
            + _what(hi, lvl - 1))


def _yout(p, lvl):
    if lvl == 0:
        return [p[0]]
    n = len(p) // 3
    a, b, c = _yout(p[:n], lvl - 1), _yout(p[n:2 * n], lvl - 1), _yout(p[2 * n:], lvl - 1)
    return [u + v for u, v in zip(a, b)] + [u + v for u, v in zip(b, c)]


def _raw_tap(j, lvl):
    tap = 0
    for k in range(lvl):
        dgt = (j // 3 ** (lvl - 1 - k)) % 3
        if dgt == 1:
            return None
        if dgt == 2:
            tap += 1 << (lvl - 1 - k)
    return tap


def unpk(v):
    return pltpu.bitcast(v, BF16)


def _gelu(x):
    c = math.sqrt(2.0 / math.pi)
    return 0.5 * x * (1.0 + jnp.tanh(c * (x + 0.044715 * (x * x * x))))


def _kernel(x_hbm, w1_hbm, w2_hbm, g_hbm, wf_hbm, wg_hbm, wo_hbm, o_hbm,
            xp, xh1, xh2, wa, wb, acca, accb, tmp, ys, fs, fe_ref, ge_ref,
            g_v, wf_v, wg_v, wo_v, ob, sem_w, sem_m, sem_x, sem_o):
    B, T, _ = x_hbm.shape
    T1 = T // 2
    T2 = T1 // 2
    U = g_hbm.shape[1]

    K = w1_hbm.shape[0]

    ww = (wa, wb)

    class _Copies:
        def __init__(self, cps):
            self.cps = cps

        def start(self):
            for c in self.cps:
                c.start()

        def wait(self, ph):
            for c in (self.cps[:1] if ph == 0 else self.cps[1:]):
                c.wait()

    def w_copy(w_hbm, wr, dt, si):
        c0 = dt * 128 if isinstance(dt, int) else pl.multiple_of(dt * 128, 128)
        n = K // 2
        w2d = w_hbm.at[pl.ds(0, 2 * n)].reshape(n, 2, D, D)
        return _Copies([
            pltpu.make_async_copy(w2d.at[:, 1, :, pl.ds(c0, 128)],
                                  wa.at[pl.ds(wr + 16 * dt, n)], sem_w.at[3 * si]),
            pltpu.make_async_copy(w2d.at[:, 0, :, pl.ds(c0, 128)],
                                  wb.at[pl.ds(wr + 16 * dt, n)], sem_w.at[3 * si + 1]),
            pltpu.make_async_copy(w_hbm.at[2 * n, :, pl.ds(c0, 128)],
                                  wb.at[wr + 16 * dt + n], sem_w.at[3 * si + 2]),
        ])

    xu = x_hbm.bitcast(jnp.uint32)
    x_cps = [pltpu.make_async_copy(xu.at[b, :, pl.ds(ct * 128, 128)],
                                   xp.at[b * NT + ct, pl.ds(8, T1)], sem_x.at[b * NT + ct])
             for b in range(B) for ct in range(NT)]
    small = [pltpu.make_async_copy(s, d_, sem_m.at[1 + k]) for k, (s, d_) in enumerate(
        ((wf_hbm, wf_v), (g_hbm, g_v), (wg_hbm, wg_v), (wo_hbm, wo_v)))]

    z0 = 8 + (T1 // 8) * 8
    for bc in range(B * NT):
        xp[bc, 0:8] = jnp.zeros((8, 128), jnp.uint32)
        xp[bc, z0:] = jnp.zeros((xp.shape[1] - z0, 128), jnp.uint32)
    for c_ in x_cps:
        c_.start()

    zb = jnp.zeros((512, 128), BF16)
    for dt in range(NT):
        wa[WR1 + 16 * dt + 15] = zb
        wa[WR2 + 16 * dt + 15] = zb
    zf = jnp.zeros((8, 128), F32)
    for ct in range(NT):
        for j in range(M1):
            for b in range(B):
                ys[ct, j, b, 0:8] = zf
                ys[ct, j, b, 8 + NB:16 + NB] = zf
    accb[...] = jnp.zeros(accb.shape, F32)

    for c_ in x_cps:
        c_.wait()
    w_copy(w1_hbm, WR1, 0, 0).start()
    hm = M1 // 2
    nw = 2 * hm - 1

    def xd(bc, ph, r, l):
        v = xp[bc, pl.ds(r * M1 + l + 1 - ph, 8, stride=M1), :]
        return pltpu.bitcast(v & jnp.uint32(0xFFFF0000) if ph else v << 16, F32)

    def xh1_top(bc, c):
        for r in range(0, NB, 8):
            for ph in range(2):
                for l in range(nw):
                    mid = xd(bc, ph, r, hm + l)
                    tmp[bc, ph, 0, l, r:r + 8] = xd(bc, ph, r, l) - mid
                    tmp[bc, ph, 1, l, r:r + 8] = mid
                    tmp[bc, ph, 2, l, r:r + 8] = xd(bc, ph, r, 2 * hm + l) - mid
        return c

    jax.lax.fori_loop(0, B * NT, xh1_top, 0)
    w_copy(w1_hbm, WR1, 1, 1).start()

    def xh1_rest(i, c):
        bc, hf = i // 2, i % 2
        b, ct = bc // NT, bc % NT
        r = pl.multiple_of(hf * 16, 16)
        r0 = pl.multiple_of(b * NB + hf * 16, 16)
        for ph in range(2):
            for q in range(3):
                dl = [tmp[bc, ph, q, l, pl.ds(r, 16)] for l in range(nw)]
                for j, v in enumerate(_xhat(dl, L1 - 1)):
                    xh1[ph, q * (R1 // 3) + j, ct, pl.ds(r0, 16)] = v.astype(BF16)
        return c

    jax.lax.fori_loop(0, B * NT * 2, xh1_rest, 0)

    def wt_piece(wr, lvl, dt, ph, buf, p):
        rs = slice(16 * p, 16 * p + 16)
        m = 1 << lvl
        ng = 16 // m
        nr = 3 ** lvl
        for g in range(ng):
            def ld(a):
                return ww[ph][wr + 16 * dt + g * m + a, rs, :].astype(F32)
            for j, v in enumerate(_what([ld(a) for a in range(m)], lvl)):
                if _raw_tap(j, lvl) is None:
                    ww[ph][WH0 + j * ng + g, rs, :] = v.astype(BF16)

    def mm_product(wr, xh, lvl, dt, ph, buf, ab, j):
        m = 1 << lvl
        ng = 16 // m
        raw = _raw_tap(j, lvl)
        res = None
        for g in range(ng):
            lhs = jnp.concatenate([unpk(xh.bitcast(jnp.uint32)[ph, j * ng + g, ct]) for ct in range(NT)], axis=1)
            if raw is not None:
                rhs = unpk(ww[ph].bitcast(jnp.uint32)[wr + 16 * dt + g * m + raw])
            else:
                rhs = unpk(ww[ph].bitcast(jnp.uint32)[WH0 + j * ng + g])
            t = jnp.dot(lhs, rhs, preferred_element_type=F32)
            res = t if res is None else res + t
        if ph == 0:
            acca[j] = res
        else:
            accb[j] = acca[j] + res

    rowid = jax.lax.broadcasted_iota(jnp.int32, (16, 128), 0)

    def epi1(ct, ab, b, hf):
        r0 = b * NB + hf * 8
        y = _yout([accb[j, r0:r0 + 8] for j in range(R1)], L1)
        nfull1 = T1 // M1
        rem1 = T1 % M1
        for j in range(M1):
            h = _gelu(y[j])
            nvalid = nfull1 + (1 if j < rem1 else 0)
            if nvalid < hf * 8 + 8:
                h = jnp.where(rowid[:8] + hf * 8 < nvalid, h, 0.0)
            ys[ct, j, b, 8 + hf * 8:16 + hf * 8] = h

    def xhat2(ct, ph, g, b, hf):
        dd = []
        for l in range(2 * M2 - 1):
            k = 2 * l + (2 if ph == 0 else 1) + 2 * M2 * (g - 1)
            sh = k // M1
            dd.append(ys[ct, k % M1, b, pl.ds(8 + sh + hf * 16, 16), :])
        r0 = b * NB + hf * 16
        for j, v in enumerate(_xhat(dd, L2)):
            xh2[ph, j * G2 + g, ct, r0:r0 + 16] = v.astype(BF16)

    def epi2(ct, ab):
        y = _yout([accb[j] for j in range(R2)], L2)
        for j in range(M2):
            fs[ct, j] = _gelu(y[j]).astype(BF16)

    def interleave(main, fill, head=0):
        for f in main[:head]:
            f()
        main = main[head:]
        nm, nf = len(main), len(fill)
        k = 0
        for i, f in enumerate(main):
            f()
            while k < nf and k * nm < (i + 1) * nf:
                fill[k]()
                k += 1
        while k < nf:
            fill[k]()
            k += 1

    def mix(a, b):
        out = []
        interleave([P(out.append, f) for f in a], [P(out.append, f) for f in b])
        return out

    nreg = [0]

    def region(i, f):
        nreg[0] += 1
        pl.when(i < 2 * NT + nreg[0])(f)

    P = functools_partial
    ord1 = sorted(range(R1), key=lambda j: _raw_tap(j, L1) is None)
    ord2 = sorted(range(R2), key=lambda j: _raw_tap(j, L2) is None)
    nraw1, nraw2 = 0, 0

    w_copy(w1_hbm, WR1, 0, 0).wait(0)
    for p in range(D // 16):
        wt_piece(WR1, L1, 0, 0, 0, p)

    def conv1_body(dt, c):
        ab = dt % 2
        dn = jnp.minimum(dt + 1, NT - 1)
        dp = jnp.maximum(dt - 1, 0)
        d2 = jnp.minimum(dt + 2, NT - 1)

        @pl.when(dt + 2 < NT)
        def _():
            w_copy(w1_hbm, WR1, d2, d2).start()

        @pl.when(dt + 2 == NT)
        def _():
            for c_ in small:
                c_.start()
            w_copy(w2_hbm, WR2, 0, NT).start()

        @pl.when(dt + 1 == NT)
        def _():
            for q in range(1, NT):
                w_copy(w2_hbm, WR2, q, NT + q).start()

        w_copy(w1_hbm, WR1, dt, dt).wait(1)

        fill = [P(wt_piece, WR1, L1, dt, 1, 1, p) for p in range(D // 16)]
        fill = mix(fill, [P(epi1, dp, 1 - ab, b, hf) for b in range(B) for hf in range(4)])
        region(dt, lambda: interleave([P(mm_product, WR1, xh1, L1, dt, 0, 0, ab, j) for j in ord1], fill, nraw1))
        @pl.when(dt + 1 < NT)
        def _():
            w_copy(w1_hbm, WR1, dn, dn).wait(0)

        fill = [P(wt_piece, WR1, L1, dn, 0, 0, p) for p in range(D // 16)]
        fill = mix(fill, [P(xhat2, dp, ph, g, b, hf) for ph in range(2) for g in range(G2)
                          for b in range(B) for hf in range(2)])
        region(dt, lambda: interleave([P(mm_product, WR1, xh1, L1, dt, 1, 1, ab, j) for j in ord1], fill, nraw1))
        return c

    jax.lax.fori_loop(0, NT, conv1_body, 0)

    for b in range(B):
        for hf in range(4):
            epi1(NT - 1, (NT - 1) % 2, b, hf)
    for ph in range(2):
        for g in range(G2):
            for b in range(B):
                for hf in range(2):
                    xhat2(NT - 1, ph, g, b, hf)

    w_copy(w2_hbm, WR2, 0, NT).wait(0)
    for p in range(D // 16):
        wt_piece(WR2, L2, 0, 0, 0, p)

    def conv2_body(dt, c):
        ab = dt % 2
        dn = jnp.minimum(dt + 1, NT - 1)
        dp = jnp.maximum(dt - 1, 0)
        w_copy(w2_hbm, WR2, dt, NT + dt).wait(1)

        fill = [P(wt_piece, WR2, L2, dt, 1, 1, p) for p in range(D // 16)]
        fill.insert(0, P(epi2, dp, 1 - ab))
        region(dt, lambda: interleave([P(mm_product, WR2, xh2, L2, dt, 0, 0, ab, j) for j in ord2], fill, nraw2))
        @pl.when(dt + 1 < NT)
        def _():
            w_copy(w2_hbm, WR2, dn, NT + dn).wait(0)

        fill = [P(wt_piece, WR2, L2, dn, 0, 0, p) for p in range(D // 16)]
        region(dt, lambda: interleave([P(mm_product, WR2, xh2, L2, dt, 1, 1, ab, j) for j in ord2], fill, nraw2))
        return c

    jax.lax.fori_loop(0, NT, conv2_body, 0)
    epi2(NT - 1, (NT - 1) % 2)

    for c_ in small:
        c_.wait()
    f2 = jnp.concatenate([fs[ct].reshape(M2 * B * NB, 128) for ct in range(NT)], axis=1)
    fe_ref[...] = jnp.dot(f2, wf_v[...], preferred_element_type=F32)
    ge_ref[...] = jnp.dot(g_v[...].reshape(B * U, D), wg_v[...], preferred_element_type=F32)

    TC = 64
    chunks = [(t0, min(TC, T2 - t0)) for t0 in range(0, T2, TC)]

    def o_copy(b, k):
        t0, tc = chunks[k]
        return pltpu.make_async_copy(ob.at[b, pl.ds(t0, tc)], o_hbm.at[b, pl.ds(t0, tc)],
                                     sem_o.at[b * len(chunks) + k])

    def joint_body(b, c):
        geb = ge_ref[pl.ds(pl.multiple_of(b * U, U), U)]
        for k, (t0, tc) in enumerate(chunks):
            rows = []
            for t in range(t0, t0 + tc):
                r = (t % M2) * (B * NB) + t // M2
                rows.append(jnp.tanh(fe_ref[pl.ds(b * NB + r, 1), :] + geb).astype(BF16))
            jm = jnp.concatenate(rows, axis=0)
            res = jnp.dot(jm, wo_v[...], preferred_element_type=F32)
            ob[b, t0:t0 + tc] = res.astype(BF16).reshape(tc, U, D)
            o_copy(b, k).start()
        return c

    jax.lax.fori_loop(0, B, joint_body, 0)
    for b in range(B):
        for k in range(len(chunks)):
            o_copy(b, k).wait()


def functools_partial(f, *a):
    return lambda: f(*a)


@jax.jit
def pallas_standalone__seq2seq_rnn_t_joint__speech_kernel(
    x: jax.Array,
    w1: jax.Array,
    w2: jax.Array,
    g: jax.Array,
    w_f: jax.Array,
    w_g: jax.Array,
    w_o: jax.Array,
):
    B, T, Dm = x.shape
    K = w1.shape[0]
    U = g.shape[1]
    assert Dm == D and K == 31 and B == 2 and T % 4 == 0
    T1 = T // 2
    T2 = T1 // 2
    assert -(-T1 // M1) == NB and -(-T2 // M2) == NB
    any_spec = pl.BlockSpec(memory_space=pl.ANY)
    n_out = B * (-(-T2 // 64))
    scratch = [
        pltpu.VMEM((B * NT, M1 * NB + 32, 128), jnp.uint32),
        pltpu.VMEM((2, R1, NT, B * NB, 128), BF16),
        pltpu.VMEM((2, R2 * G2, NT, B * NB, 128), BF16),
        pltpu.VMEM((WH0 + RH, D, 128), BF16),
        pltpu.VMEM((WH0 + RH, D, 128), BF16),
        pltpu.VMEM((R1, B * NB, 128), F32),
        pltpu.VMEM((R1, B * NB, 128), F32),
        pltpu.VMEM((B * NT, 2, 3, M1 - 1, NB, 128), F32),
        pltpu.VMEM((NT, M1, B, NB + 16, 128), F32),
        pltpu.VMEM((NT, M2, B * NB, 128), BF16),
        pltpu.VMEM((M2 * B * NB, D), F32),
        pltpu.VMEM((B * U, D), F32),
        pltpu.VMEM((B, U, D), BF16),
        pltpu.VMEM((D, D), BF16),
        pltpu.VMEM((D, D), BF16),
        pltpu.VMEM((D, D), BF16),
        pltpu.VMEM((B, T2, U, D), BF16),
        pltpu.SemaphoreType.DMA((24,)),
        pltpu.SemaphoreType.DMA((5,)),
        pltpu.SemaphoreType.DMA((B * NT,)),
        pltpu.SemaphoreType.DMA((n_out,)),
    ]
    return pl.pallas_call(
        _kernel,
        in_specs=[any_spec] * 7,
        out_specs=any_spec,
        out_shape=jax.ShapeDtypeStruct((B, T2, U, D), BF16),
        scratch_shapes=scratch,
        compiler_params=pltpu.CompilerParams(vmem_limit_bytes=116 * 1024 * 1024),
    )(x, w1, w2, g, w_f, w_g, w_o)
```
